```python
import os as _os
_os.environ.setdefault("JAX_PLATFORMS", "cpu")
import jax
import jax.numpy as jnp

def _softmax(x, axis=-1):
    return jax.nn.softmax(x, axis=axis)
def _gelu(x):
    return jax.nn.gelu(x, approximate=True)
def _silu(x):
    return jax.nn.silu(x)
def _sigmoid(x):
    return jax.nn.sigmoid(x)
def _layernorm(x, axis=-1, eps=1e-5):
    m = jnp.mean(x, axis=axis, keepdims=True)
    v = jnp.var(x, axis=axis, keepdims=True)
    return (x - m) / jnp.sqrt(v + eps)
def _scatter_add(tgt, idx, src, axis=0):
    return tgt.at[idx].add(src)
def _segment_sum(src, seg, n):
    return jax.ops.segment_sum(src, seg, n)
class _Rng:
    def __init__(self, key):
        self._k = key
    def _next(self):
        self._k, sub = jax.random.split(self._k)
        return sub
    def normal(self, shape):
        return jax.random.normal(self._next(), shape, dtype=jnp.bfloat16)
    def randint(self, lo, hi, shape):
        return jax.random.randint(self._next(), shape, lo, hi, dtype=jnp.int32)
    def uniform(self, shape, lo=0.0, hi=1.0):
        return jax.random.uniform(self._next(), shape, jnp.bfloat16, lo, hi)
    def permutation(self, n):
        return jax.random.permutation(self._next(), n)


kernel_name = 'concat_heads__sliding_block_cached__sliding_block_cached__decode'

def setup_inputs():
    _rng = _Rng(jax.random.key(int.from_bytes(__import__("os").urandom(4), "little")))
    _w = (lambda a: (lambda t: t.astype(jnp.bfloat16) if jnp.issubdtype(t.dtype, jnp.floating) else t)(jnp.asarray(a)))
    def _A_setup():
        B, Sq, D = 1, 1, 640
        Hq, Hkv, Sk, Dh = 32, 32, 4096, 192
        assert Hq % Hkv == 0, (Hq, Hkv)
        return {
            "x": _w((lambda *s: _rng.normal(s) * 0.8)(B, Sq, D)),
            "k_cache": _w((lambda *s: _rng.normal(s) * 0.8)(B, Hkv, Sk, Dh)),
            "v_cache": _w((lambda *s: _rng.normal(s) * 0.05)(B, Hkv, Sk, Dh)),
            "wq": _w((lambda *s: _rng.normal(s) * 0.8)(D, Hq * Dh) * (D ** -0.5)),
            "wo": _w((lambda *s: _rng.normal(s) * 0.05)(Hq * Dh, D) * ((Hq * Dh) ** -0.5)),
        }
    _A_in = _A_setup()

    def _B_setup():
        B, Sq, D = 1, 1, 640
        Hq, Hkv, Sk, Dh = 32, 32, 4096, 192
        assert Hq % Hkv == 0, (Hq, Hkv)
        return {
            "x": _w((lambda *s: _rng.normal(s) * 0.8)(B, Sq, D)),
            "k_cache": _w((lambda *s: _rng.normal(s) * 0.8)(B, Hkv, Sk, Dh)),
            "v_cache": _w((lambda *s: _rng.normal(s) * 0.05)(B, Hkv, Sk, Dh)),
            "wq": _w((lambda *s: _rng.normal(s) * 0.8)(D, Hq * Dh) * (D ** -0.5)),
            "wo": _w((lambda *s: _rng.normal(s) * 0.05)(Hq * Dh, D) * ((Hq * Dh) ** -0.5)),
        }
    _B_in = _B_setup()

    return {
        "A_x": _A_in["x"],
        "A_k_cache": _A_in["k_cache"],
        "A_v_cache": _A_in["v_cache"],
        "A_wq": _A_in["wq"],
        "A_wo": _A_in["wo"],
        "B_x": _B_in["x"],
        "B_k_cache": _B_in["k_cache"],
        "B_v_cache": _B_in["v_cache"],
        "B_wq": _B_in["wq"],
        "B_wo": _B_in["wo"],
    }

def reference(A_x, A_k_cache, A_v_cache, A_wq, A_wo, B_x, B_k_cache, B_v_cache, B_wq, B_wo):
    def _A_ref(x, k_cache, v_cache, wq, wo):
        B, Sq, D = x.shape
        Hq, Dh = 32, 192
        Hkv, Sk = k_cache.shape[1], k_cache.shape[2]
        W = min(4096, max(256, Sk // 4))
        rep = Hq // Hkv
        q = (lambda x, *d: x.transpose(*d))((x @ wq).reshape(B, Sq, Hq, Dh), 0, 2, 1, 3)
        k = jnp.repeat(k_cache[:, :, Sk - W:, :], rep, axis=1)
        v = jnp.repeat(v_cache[:, :, Sk - W:, :], rep, axis=1)
        scores = jnp.einsum("bhqd,bhkd->bhqk", q, k) * (Dh ** -0.5)
        p = _softmax(scores, axis=-1)
        o = jnp.einsum("bhqk,bhkd->bhqd", p, v)
        return (lambda x, *d: x.transpose(*d))(o, 0, 2, 1, 3).reshape(B, Sq, Hq * Dh) @ wo

    def _B_ref(x, k_cache, v_cache, wq, wo):
        B, Sq, D = x.shape
        Hq, Dh = 32, 192
        Hkv, Sk = k_cache.shape[1], k_cache.shape[2]
        W = min(4096, max(256, Sk // 4))
        rep = Hq // Hkv
        q = (lambda x, *d: x.transpose(*d))((x @ wq).reshape(B, Sq, Hq, Dh), 0, 2, 1, 3)
        k = jnp.repeat(k_cache[:, :, Sk - W:, :], rep, axis=1)
        v = jnp.repeat(v_cache[:, :, Sk - W:, :], rep, axis=1)
        scores = jnp.einsum("bhqd,bhkd->bhqk", q, k) * (Dh ** -0.5)
        p = _softmax(scores, axis=-1)
        o = jnp.einsum("bhqk,bhkd->bhqd", p, v)
        return (lambda x, *d: x.transpose(*d))(o, 0, 2, 1, 3).reshape(B, Sq, Hq * Dh) @ wo

    a = _A_ref(A_x, A_k_cache, A_v_cache, A_wq, A_wo)
    b = _B_ref(B_x, B_k_cache, B_v_cache, B_wq, B_wo)
    return jnp.concatenate([a, b], axis=-1)
```

```python
import functools
import jax
import jax.numpy as jnp
from jax import lax
from jax.experimental import pallas as pl
from jax.experimental.pallas import tpu as pltpu

H, DH, SK, W, D = 32, 192, 4096, 1024, 640
R = H * DH
OFF = SK - W
HG = 8
RG = HG * DH
NG = H // HG
SCALE = DH ** -0.5
BF, F32 = jnp.bfloat16, jnp.float32


def make(sq=4, skv=12, so=4, checks=False, compute=True):
    def kernel(ax, ak, av, awq, awo, bx, bk, bv, bwq, bwo, o_ref,
               xb, wqb, kb, vb, wob, qs, ps, os_, acc, sems):
        xs, ks, vs, wqs, wos = (ax, bx), (ak, bk), (av, bv), (awq, bwq), (awo, bwo)
        SEM_Q, SEM_K, SEM_V, SEM_O = 0, 1, 2, 3

        def cp(src, dst, sem, prio):
            pltpu.make_async_copy(src, dst, sems.at[sem]).start(priority=prio)

        def wait(buf, sem):
            pltpu.make_async_copy(buf, buf, sems.at[sem]).wait()

        n1 = D // 8 // sq
        def p1(i, _):
            for c in range(R // 1024):
                for s in range(sq):
                    row = pl.ds(pl.multiple_of(i * 8, 8) + s * (D // sq), 8)
                    col = pl.ds(c * 1024, 1024)
                    for b in range(2):
                        cp(wqs[b].at[row, col], wqb.at[b, row, col], SEM_Q, b)
        lax.fori_loop(0, n1, p1, None)
        for b in range(2):
            cp(xs[b].at[0], xb.at[b], SEM_Q, b)

        def kv_issue(srcs, dst, sem, i, n):
            m = R // 8 // skv // n
            for j in range(m):
                for s in range(skv):
                    row = pl.ds(pl.multiple_of(i * (8 * m), 8) + (j * 8 + s * (R // skv)), 8)
                    for b in range(2):
                        cp(srcs[b].at[row, pl.ds(OFF, W)], dst.at[b, row, :], sem, b)

        n2 = 64
        lag = 4
        QC = 256
        def p2(i, _):
            kv_issue(ks, kb, SEM_K, i, n2)
            @pl.when(i == lag)
            def _():
                wait(wqb, SEM_Q)
                wait(xb, SEM_Q)
            if compute:
                @pl.when(jnp.logical_and(i >= lag, i < lag + 2 * R // QC))
                def _():
                    j = i - lag
                    b = j // (R // QC)
                    c = pl.ds(pl.multiple_of((j % (R // QC)) * QC, QC), QC)
                    x8 = jnp.broadcast_to(xb[b], (8, D))
                    qs[b, :, c] = jnp.dot(x8, wqb[b, :, c], preferred_element_type=F32)
        lax.fori_loop(0, n2, p2, None)

        row_lo = lax.broadcasted_iota(jnp.int32, (HG, RG), 0) * DH
        col = lax.broadcasted_iota(jnp.int32, (HG, RG), 1)
        SC = 256
        def p3(i, _):
            kv_issue(vs, vb, SEM_V, i, n2)
            @pl.when(i == lag)
            def _():
                wait(kb, SEM_K)
            if compute:
                nc = W // SC
                @pl.when(jnp.logical_and(i >= lag, i < lag + 2 * NG * nc))
                def _():
                    j = i - lag
                    bg = j // nc
                    b, g = bg // NG, bg % NG
                    r = pl.ds(pl.multiple_of(g * RG, RG), RG)
                    c = pl.ds(pl.multiple_of((j % nc) * SC, SC), SC)
                    diag = jnp.logical_and(col >= row_lo, col < row_lo + DH)
                    qbd = jnp.where(diag, qs[b, :, r], 0.0).astype(BF)
                    ps[bg, :, c] = jnp.dot(qbd, kb[b, r, c], preferred_element_type=F32) * SCALE
                @pl.when(i == lag + 2 * NG * nc)
                def _():
                    s = ps[...]
                    e = jnp.exp(s - jnp.max(s, axis=-1, keepdims=True))
                    ps[...] = e / jnp.sum(e, axis=-1, keepdims=True)
        lax.fori_loop(0, n2, p3, None)

        n4 = 48
        rs = R // so
        ri = rs // n4
        ipb = 128 // ri
        nblk = n4 // ipb
        acc[...] = jnp.zeros_like(acc)

        def wo_block(k):
            v = wob.at[:, :, pl.ds(pl.multiple_of(k * 128, 128), 128), :]
            wait(v, SEM_O + k)
            if compute:
                for b in range(2):
                    part = acc[b]
                    for s in range(so):
                        r = pl.ds(pl.multiple_of(k * 128, 128) + s * rs, 128)
                        part += jnp.dot(os_[b, :, r].astype(BF), wob[b, s, pl.ds(pl.multiple_of(k * 128, 128), 128), :],
                                        preferred_element_type=F32)
                    acc[b] = part

        PC = 384
        npv = 2 * R // PC
        def p4(i, _):
            for j in range(ri // 16):
                for s in range(so):
                    r0 = pl.multiple_of(i * ri, 16) + j * 16
                    for b in range(2):
                        cp(wos[b].at[pl.ds(r0 + s * rs, 16), :], wob.at[b, s, pl.ds(r0, 16), :], SEM_O + i // ipb, b)
            @pl.when(i == lag)
            def _():
                wait(vb, SEM_V)
            if compute:
                @pl.when(jnp.logical_and(i >= lag, i < lag + npv))
                def _():
                    j = i - lag
                    b = j // (R // PC)
                    jj = j % (R // PC)
                    r = pl.ds(pl.multiple_of(jj * PC, PC), PC)
                    bg = j // (RG // PC)
                    p = ps[bg].astype(BF)
                    o = lax.dot_general(p, vb[b, r, :], (((1,), (1,)), ((), ())), preferred_element_type=F32)
                    cc = lax.broadcasted_iota(jnp.int32, (HG, PC), 1) + (j % (RG // PC)) * PC
                    lo = lax.broadcasted_iota(jnp.int32, (HG, PC), 0) * DH
                    o = jnp.where(jnp.logical_and(cc >= lo, cc < lo + DH), o, 0.0)
                    os_[b, :, r] = jnp.broadcast_to(jnp.sum(o, axis=0, keepdims=True), (HG, PC))
            @pl.when(i >= n4 - (nblk - 2))
            def _():
                wo_block(i - (n4 - (nblk - 2)))
        assert lag + npv <= n4 - (nblk - 2)
        lax.fori_loop(0, n4, p4, None)
        lax.fori_loop(nblk - 2, nblk, lambda k, _: wo_block(k), None)
        for b in range(2):
            o_ref[0, :, pl.ds(b * D, D)] = acc[b, pl.ds(0, 1), :].astype(o_ref.dtype)

    def fn(ax, ak, av, awq, awo, bx, bk, bv, bwq, bwo):
        t = lambda a: jnp.swapaxes(a, 2, 3).reshape(R, SK)
        any_ = pl.BlockSpec(memory_space=pl.ANY)
        return pl.pallas_call(
            kernel,
            in_specs=[any_] * 10,
            out_specs=pl.BlockSpec(memory_space=pltpu.VMEM),
            out_shape=jax.ShapeDtypeStruct((1, 1, 2 * D), BF),
            scratch_shapes=[
                pltpu.VMEM((2, 1, D), BF),
                pltpu.VMEM((2, D, R), BF),
                pltpu.VMEM((2, R, W), BF),
                pltpu.VMEM((2, R, W), BF),
                pltpu.VMEM((2, so, R // so, D), BF),
                pltpu.VMEM((2, HG, R), F32),
                pltpu.VMEM((2 * NG, HG, W), F32),
                pltpu.VMEM((2, HG, R), F32),
                pltpu.VMEM((2, HG, D), F32),
                pltpu.SemaphoreType.DMA((3 + R // so // 128,)),
            ],
            compiler_params=pltpu.CompilerParams(
                vmem_limit_bytes=110 * 2 ** 20,
                disable_semaphore_checks=not checks, disable_bounds_checks=not checks),
        )(ax, t(ak), t(av), awq, awo, bx, t(bk), t(bv), bwq, bwo)
    return fn


_fn = make()


@jax.jit
def pallas_concat_heads__sliding_block_cached__sliding_block_cached__decode_kernel(
    A_x, A_k_cache, A_v_cache, A_wq, A_wo, B_x, B_k_cache, B_v_cache, B_wq, B_wo):
    return _fn(A_x, A_k_cache, A_v_cache, A_wq, A_wo, B_x, B_k_cache, B_v_cache, B_wq, B_wo)
```

```python
import functools

import jax
import jax.numpy as jnp
from jax import lax
import jax.experimental.pallas as pl
import jax.experimental.pallas.tpu as pltpu

H, DH, SK, D = 32, 192, 4096, 640
W = min(4096, max(256, SK // 4))
R = H * DH
SCALE = DH ** -0.5
BF, F32 = jnp.bfloat16, jnp.float32

KV_STRIPES, KV_PIECES, KV_ITERS, KV_GROUP = 96, 12, 64, 6
W_STRIPES, W_ITERS, W_GROUP = 15, 32, 5
SIDE_LAG = 2
KV_LAG, W_LAG = 8, 5
LAST_GROUPS = (7, 4, 2, 2)

SEM_X, SEM_WQ, SEM_K, SEM_V, SEM_WO_A, SEM_WO_B = 0, 1, 3, 5, 7, 8
NUM_SEMS = SEM_WO_B + W_ITERS - 1 + len(LAST_GROUPS)


def _copy_order(pieces, group):
    order = []
    for g in range(0, pieces, group):
        main = [(g + i, False, 0) for i in range(1, group)]
        mid = group // 2
        order += [(g, True, 0)] + main[:mid] + [(g, True, 1)] + main[mid:]
    return order


def _w_stripe(piece):
    return -2 * piece % W_STRIPES


def _div(x, d):
    if isinstance(x, int):
        return x // d
    return lax.shift_right_logical(x * (2048 // d + 1), 11)


def _ds(start, size, multiple):
    if not isinstance(start, int):
        start = pl.multiple_of(start, multiple)
    return pl.ds(start, size)


def _kernel(a_x, a_k, a_v, a_wq, a_wo, b_x, b_k, b_v, b_wq, b_wo, o_ref,
            x_buf, wq_buf, k_buf, v_buf, wo_buf, q_buf, p_buf, o_buf, acc_buf, sems):

    def start(src, dst, sem, side):
        pltpu.make_async_copy(src, dst, sems.at[sem]).start(priority=0 if side else 1)

    def wait(buf, sem):
        pltpu.make_async_copy(buf, buf, sems.at[sem]).wait()

    def wq_copies(b, it):
        its = (it, (it - SIDE_LAG) & (W_ITERS - 1))
        for piece, side, half in _copy_order(W_STRIPES, W_GROUP):
            s = _w_stripe(piece)
            p = its[side] + W_ITERS * (s % 3)
            row = _div(p, 6)
            n = 512 if side else 1024
            idx = (s // 3, _ds(row * 8, 8, 8), _ds((p - row * 6) * 1024 + half * n, n, n))
            start((a_wq, b_wq)[b].at[idx], wq_buf.at[(b,) + idx], SEM_WQ + b, side)

    def kv_copies(srcs, buf, sem, b, it):
        its = (it, (it - SIDE_LAG) & (KV_ITERS - 1))
        for piece, side, half in _copy_order(KV_PIECES, KV_GROUP):
            i = its[side]
            s = ((i + 7 * (piece % 2)) & 7) * KV_PIECES + piece
            rows = _ds(lax.shift_right_logical(i, 3) * 8, 8, 8)
            n = W // 2 if side else W
            start(srcs[b].at[s, rows, pl.ds(SK - W + half * n, n)],
                  buf.at[b, s, rows, pl.ds(half * n, n)], sem + b, side)

    def wo_copy(b, i, piece, side, half):
        sem = SEM_WO_A
        if b == 1:
            group = sum(piece >= sum(LAST_GROUPS[:g + 1]) for g in range(len(LAST_GROUPS)))
            sem = SEM_WO_B + i + jnp.where(i == W_ITERS - 1, group, 0)
        n = 32 if side else 64
        rows = pl.ds(half * n, n)
        start((a_wo, b_wo)[b].at[_w_stripe(piece), i, rows], wo_buf.at[b, i, piece, rows], sem, side)

    def wo_copies(b, it):
        its = (it, (it - SIDE_LAG) & (W_ITERS - 1))
        for piece, side, half in _copy_order(W_STRIPES, W_GROUP):
            copy = functools.partial(wo_copy, b, its[side], piece, side, half)
            if b == 1 and side:
                pl.when(it >= SIDE_LAG)(copy)
            else:
                copy()

    def q_step(b, j):
        cols = _ds(j * 256, 256, 256)
        x = jnp.broadcast_to(x_buf[b], (8, D))
        w = wq_buf[b, :, :, cols].reshape(D, 256)
        q_buf[b, :, cols] = jnp.dot(x, w, preferred_element_type=F32)

    def score_step(b, j):
        g = lax.shift_right_logical(j, 3)
        keys = _ds((j & 7) * 128, 128, 128)
        first = lax.broadcasted_iota(jnp.int32, (8, 8 * DH), 0) * DH
        col = lax.broadcasted_iota(jnp.int32, (8, 8 * DH), 1)
        q = q_buf[b, :, _ds(g * (8 * DH), 8 * DH, 8 * DH)]
        q = jnp.where(jnp.logical_and(col >= first, col < first + DH), q, 0.0).astype(BF)
        k = k_buf[b, pl.ds(24 * g, 24), :, keys].reshape(8 * DH, 128)
        p_buf[b, _ds(g * 8, 8, 8), keys] = jnp.dot(q, k, preferred_element_type=F32) * SCALE

    def softmax_step(b, g):
        heads = _ds(g * 8, 8, 8)
        s = p_buf[b, heads, :]
        e = jnp.exp(s - jnp.max(s, axis=-1, keepdims=True))
        p_buf[b, heads, :] = e / jnp.sum(e, axis=-1, keepdims=True)

    def pv_step(b, j):
        for u in range(4):
            s = 4 * j + u
            p = p_buf[b, pl.ds(_div(s, 3), 1), :]
            o = jnp.sum(v_buf[b, s].astype(F32) * p, axis=-1, keepdims=True)
            o_buf[b, pl.ds(s * 8, 8)] = jnp.broadcast_to(o, (64, 128)).reshape(8, 8, 128)

    def out_fma(b, it, acc, pieces):
        rows = [_div(8 * it + m, 5) for m in range(12)]
        for piece in pieces:
            s = _w_stripe(piece)
            w = wo_buf[b, it, piece].astype(F32)
            for j in range(8):
                o = o_buf[b, rows[s % 5 + j] + (256 * (s // 5) + 51 * (s % 5))]
                acc[(s + j) % 5] += w[8 * j:8 * j + 8] * o

    def out_step(b, it):
        if b == 1:
            wait(wo_buf.at[1, it], SEM_WO_B + it)
        acc = [acc_buf[b, z] for z in range(5)]
        out_fma(b, it, acc, range(W_STRIPES))
        for z in range(5):
            acc_buf[b, (z + 2) % 5] = acc[z]

    def out_store(b, it, acc):
        out = [jnp.sum(acc[(c - 3 * it) % 5], axis=0, keepdims=True) for c in range(5)]
        o_ref[0, :, pl.ds(b * D, D)] = jnp.concatenate(out, axis=1).astype(o_ref.dtype)

    def stream(iters, copies, lag, landed, *work):
        @pl.loop(0, iters)
        def _(it):
            copies(it)
            pl.when(it == lag)(functools.partial(wait, *landed))
            first = lag
            for steps, step in work:
                active = jnp.logical_and(it >= first, it < first + steps)
                pl.when(active)(functools.partial(step, it - first))
                first += steps
            assert first <= iters

    part = functools.partial
    k_copies = part(kv_copies, (a_k, b_k), k_buf, SEM_K)
    v_copies = part(kv_copies, (a_v, b_v), v_buf, SEM_V)

    wq_copies(0, 0)
    for b, x in enumerate((a_x, b_x)):
        start(x.at[0], x_buf.at[b], SEM_X, True)
    pl.loop(1, W_ITERS)(part(wq_copies, 0))
    wait(x_buf, SEM_X)
    acc_buf[...] = jnp.zeros_like(acc_buf)

    stream(W_ITERS, part(wq_copies, 1), W_LAG, (wq_buf.at[0], SEM_WQ), (24, part(q_step, 0)))
    stream(KV_ITERS, part(k_copies, 0), KV_LAG, (wq_buf.at[1], SEM_WQ + 1), (24, part(q_step, 1)))
    stream(KV_ITERS, part(k_copies, 1), KV_LAG, (k_buf.at[0], SEM_K),
           (32, part(score_step, 0)), (4, part(softmax_step, 0)))
    stream(KV_ITERS, part(v_copies, 0), KV_LAG, (k_buf.at[1], SEM_K + 1),
           (32, part(score_step, 1)), (4, part(softmax_step, 1)))
    stream(KV_ITERS, part(v_copies, 1), KV_LAG, (v_buf.at[0], SEM_V), (24, part(pv_step, 0)))
    stream(W_ITERS, part(wo_copies, 0), W_LAG, (v_buf.at[1], SEM_V + 1), (24, part(pv_step, 1)))

    def out_steps(it):
        out_step(0, it)
        out_step(1, it)

    rest = W_ITERS - W_LAG
    stream(W_ITERS, part(wo_copies, 1), W_LAG, (wo_buf.at[0], SEM_WO_A), (rest, out_steps))

    @pl.loop(0, W_LAG)
    def drain(i):
        @pl.when(jnp.logical_and((i & 1) == 0, i < 2 * SIDE_LAG))
        def _():
            it = W_ITERS - SIDE_LAG + lax.shift_right_logical(i, 1)
            for piece, side, half in _copy_order(W_STRIPES, W_GROUP):
                if side:
                    wo_copy(1, it, piece, side, half)
        out_step(0, rest + i)

    out_store(0, W_ITERS, [acc_buf[0, z] for z in range(5)])

    last = W_ITERS - 1
    pl.loop(rest, last)(part(out_step, 1))
    acc = [acc_buf[1, z] for z in range(5)]
    first = 0
    for g, n in enumerate(LAST_GROUPS):
        wait(wo_buf.at[1, last, pl.ds(first, n)], SEM_WO_B + last + g)
        out_fma(1, last, acc, range(first, first + n))
        first += n
    out_store(1, last, acc)


@jax.jit
def pallas_concat_heads__sliding_block_cached__sliding_block_cached__decode_kernel(
    A_x: jax.Array,
    A_k_cache: jax.Array,
    A_v_cache: jax.Array,
    A_wq: jax.Array,
    A_wo: jax.Array,
    B_x: jax.Array,
    B_k_cache: jax.Array,
    B_v_cache: jax.Array,
    B_wq: jax.Array,
    B_wo: jax.Array,
):
    def kv_view(c):
        return jnp.swapaxes(c, 2, 3).reshape(KV_STRIPES, R // KV_STRIPES, SK)

    def wq_view(w):
        return w.reshape(D // 128, 128, R)

    def wo_view(w):
        tiles = w.reshape(R // 8, 8, D // 128, 128).transpose(0, 2, 1, 3)
        return tiles.reshape(W_STRIPES, W_ITERS, 64, 128)

    return pl.pallas_call(
        _kernel,
        in_specs=[pl.BlockSpec(memory_space=pl.ANY)] * 10,
        out_specs=pl.BlockSpec(memory_space=pltpu.VMEM),
        out_shape=jax.ShapeDtypeStruct((1, 1, 2 * D), A_x.dtype),
        scratch_shapes=[
            pltpu.VMEM((2, 1, D), BF),
            pltpu.VMEM((2, D // 128, 128, R), BF),
            pltpu.VMEM((2, KV_STRIPES, R // KV_STRIPES, W), BF),
            pltpu.VMEM((2, KV_STRIPES, R // KV_STRIPES, W), BF),
            pltpu.VMEM((2, W_ITERS, W_STRIPES, 64, 128), BF),
            pltpu.VMEM((2, 8, R), F32),
            pltpu.VMEM((2, H, W), F32),
            pltpu.VMEM((2, R // 8, 8, 128), F32),
            pltpu.VMEM((2, D // 128, 8, 128), F32),
            pltpu.SemaphoreType.DMA((NUM_SEMS,)),
        ],
        compiler_params=pltpu.CompilerParams(
            vmem_limit_bytes=100 * 2 ** 20,
            disable_bounds_checks=True,
            disable_semaphore_checks=True,
        ),
    )(A_x, kv_view(A_k_cache), kv_view(A_v_cache), wq_view(A_wq), wo_view(A_wo),
      B_x, kv_view(B_k_cache), kv_view(B_v_cache), wq_view(B_wq), wo_view(B_wo))
```
